```python
import os as _os
_os.environ.setdefault("JAX_PLATFORMS", "cpu")
import jax
import jax.numpy as jnp

def _softmax(x, axis=-1):
    return jax.nn.softmax(x, axis=axis)
def _gelu(x):
    return jax.nn.gelu(x, approximate=True)
def _silu(x):
    return jax.nn.silu(x)
def _sigmoid(x):
    return jax.nn.sigmoid(x)
def _layernorm(x, axis=-1, eps=1e-5):
    m = jnp.mean(x, axis=axis, keepdims=True)
    v = jnp.var(x, axis=axis, keepdims=True)
    return (x - m) / jnp.sqrt(v + eps)
def _scatter_add(tgt, idx, src, axis=0):
    return tgt.at[idx].add(src)
def _segment_sum(src, seg, n):
    return jax.ops.segment_sum(src, seg, n)
class _Rng:
    def __init__(self, key):
        self._k = key
    def _next(self):
        self._k, sub = jax.random.split(self._k)
        return sub
    def normal(self, shape):
        return jax.random.normal(self._next(), shape, dtype=jnp.bfloat16)
    def randint(self, lo, hi, shape):
        return jax.random.randint(self._next(), shape, lo, hi, dtype=jnp.int32)
    def uniform(self, shape, lo=0.0, hi=1.0):
        return jax.random.uniform(self._next(), shape, jnp.bfloat16, lo, hi)
    def permutation(self, n):
        return jax.random.permutation(self._next(), n)


kernel_name = 'sequential_preLN__linear_attn_block__dense_activation_squared_relu__prompt'

def setup_inputs():
    _rng = _Rng(jax.random.key(int.from_bytes(__import__("os").urandom(4), "little")))
    _w = (lambda a: (lambda t: t.astype(jnp.bfloat16) if jnp.issubdtype(t.dtype, jnp.floating) else t)(jnp.asarray(a)))
    def _A_setup():
        B, S, D = 1, 2048, 576
        return {
            "x": _w((lambda *s: _rng.normal(s) * 0.05)(B, S, D)),
            "wqkv": _w((lambda *s: _rng.normal(s) * 0.1)(D, 3 * D)),
            "wo": _w((lambda *s: _rng.normal(s) * 0.05)(D, D)),
        }
    _A_in = _A_setup()

    def _B_setup():
        B, S, D, F = 1, 2048, 576, 4608
        return {
            "x": _w((lambda *s: _rng.normal(s) * 0.05)(B, S, D)),
            "w1": _w((lambda *s: _rng.normal(s) * 0.05)(D, F)),
            "b1": _w((lambda *s: _rng.normal(s) * 0.05)(F)),
            "w2": _w((lambda *s: _rng.normal(s) * 0.05)(F, D)),
            "b2": _w((lambda *s: _rng.normal(s) * 0.05)(D)),
        }
    _B_in = _B_setup()

    return {
        "A_x": _A_in["x"],
        "A_wqkv": _A_in["wqkv"],
        "A_wo": _A_in["wo"],
        "B_x": _B_in["x"],
        "B_w1": _B_in["w1"],
        "B_b1": _B_in["b1"],
        "B_w2": _B_in["w2"],
        "B_b2": _B_in["b2"],
    }

def reference(A_x, A_wqkv, A_wo, B_x, B_w1, B_b1, B_w2, B_b2):
    def _A_ref(x, wqkv, wo):
        B, S, D = x.shape
        H = 32; Dh = D // H
        qkv = (lambda x, *d: x.transpose(*d))((x @ wqkv).reshape(B, S, 3, H, Dh), 2, 0, 3, 1, 4)
        q, k, v = qkv[0], qkv[1], qkv[2]
        phi = lambda t: jnp.where(t > 0, t + 1, jnp.exp(t)) + 1e-6
        pq, pk = phi(q), phi(k)
        kv = jnp.einsum("bhsd,bhse->bhde", pk, v)
        z = jnp.einsum("bhsd->bhd", pk)
        num = jnp.einsum("bhqd,bhde->bhqe", pq, kv)
        den = jnp.einsum("bhqd,bhd->bhq", pq, z)[..., None] + 1e-6
        o = num / den
        return (lambda x, *d: x.transpose(*d))(o, 0, 2, 1, 3).reshape(B, S, D) @ wo

    def _B_ref(x, w1, b1, w2, b2):
        h = jnp.einsum("bsd,df->bsf", x, w1) + b1
        zero = jnp.zeros_like(h)
        r = jnp.where(h > zero, h, zero)
        h = r * r
        out = jnp.einsum("bsf,fd->bsd", h, w2) + b2
        return out

    x = A_x
    h = x + _A_ref(_layernorm(x, axis=-1), A_wqkv, A_wo)
    h2 = h + _B_ref(_layernorm(h, axis=-1), B_w1, B_b1, B_w2, B_b2)
    return h2
```

```python
import functools
import jax
import jax.numpy as jnp
from jax import lax
import jax.experimental.pallas as pl
import jax.experimental.pallas.tpu as pltpu

S, D, F, H, DH = 2048, 576, 4608, 32, 18
KP = 640
bf = jnp.bfloat16
f32 = jnp.float32
NN = (((1,), (0,)), ((), ()))
NT = (((1,), (1,)), ((), ()))

T1 = 256
T2 = 256
FC = 512


def _dot(a, b, dims=NN):
    return lax.dot_general(a, b, dims, preferred_element_type=f32)


def _ln_T(x):
    m = jnp.sum(x, axis=0, keepdims=True) * (1.0 / D)
    xc = x - m
    v = jnp.sum(xc * xc, axis=0, keepdims=True) * (1.0 / D)
    return xc * lax.rsqrt(v + 1e-5)


def _phi(t):
    return jnp.where(t > 0, t + 1.0, jnp.exp(t)) + 1e-6


def _head_of(idx):
    return lax.shift_right_logical(idx * 3641, 16)


def kern(x_hbm, wqkv_hbm, wo_hbm, w1_hbm, b1_hbm, w2T_hbm, b2_hbm, out_hbm,
         x_v, wqkv_v, wo_v, w1_v, b1_v, w2T_v, b2_v,
         wqkT_v, woT_v, w1T_v, g_v, pq_v, kvbd_v, mT_v, zsel_v, b2c_v, out_v,
         sem_x, sem_w, sem_o):
    nb1 = S // T1
    nb2 = S // T2

    def xcopy(i):
        return pltpu.make_async_copy(x_hbm.at[:, pl.ds(i * T1, T1)], x_v.at[:, pl.ds(i * T1, T1)], sem_x.at[i])
    c_wqk = pltpu.make_async_copy(wqkv_hbm.at[:, pl.ds(0, 1152)], wqkv_v.at[:, pl.ds(0, 1152)], sem_w.at[0])
    c_wv = pltpu.make_async_copy(wqkv_hbm.at[:, pl.ds(1152, 576)], wqkv_v.at[:, pl.ds(1152, 576)], sem_w.at[1])
    c_wo = pltpu.make_async_copy(wo_hbm, wo_v, sem_w.at[2])
    c_w1 = pltpu.make_async_copy(w1_hbm, w1_v, sem_w.at[3])
    c_w2 = pltpu.make_async_copy(w2T_hbm, w2T_v, sem_w.at[4])
    c_b1 = pltpu.make_async_copy(b1_hbm, b1_v, sem_w.at[5])
    c_b2 = pltpu.make_async_copy(b2_hbm, b2_v, sem_w.at[6])

    c_wqk.start()
    xcopy(0).start()
    c_wqk.wait()
    for i in range(1, nb1):
        xcopy(i).start()
    c_wv.start(); c_wo.start(); c_b1.start(); c_b2.start(); c_w1.start()
    for j in range(9):
        wqkT_v[j * 128:(j + 1) * 128, :] = wqkv_v[:, j * 128:(j + 1) * 128].T

    ones_blk = (lax.broadcasted_iota(jnp.int32, (64, T1), 0) == 0).astype(bf)
    for i in range(nb1):
        xcopy(i).wait()
        if i == 1:
            c_w2.start()
        x = x_v[:, i * T1:(i + 1) * T1].astype(f32)
        xn = _ln_T(x).astype(bf)
        qk = _dot(wqkT_v[...], xn)
        pq_v[:, i * T1:(i + 1) * T1] = _phi(qk[:D]).astype(bf)
        pk = _phi(qk[D:]).astype(bf)
        xe = jnp.concatenate([xn, ones_blk], axis=0)
        g = _dot(pk, xe, NT)
        if i == 0:
            g_v[...] = g
        else:
            g_v[...] += g

    c_wv.wait(); c_wo.wait(); c_b1.wait(); c_b2.wait(); c_w1.wait()
    for j in range(5):
        lo = 5 * 128 if False else 0
        if j < 4:
            woT_v[j * 128:(j + 1) * 128, :] = wo_v[:, j * 128:(j + 1) * 128].T
        else:
            woT_v[512:576, :] = wo_v[:, 448:576].T[64:, :]
    for j in range(F // 128):
        ext = (lax.broadcasted_iota(jnp.int32, (64, 128), 0) == 0)
        ext = jnp.where(ext, jnp.broadcast_to(b1_v[j:j + 1, :].astype(f32), (64, 128)), 0.0).astype(bf)
        blk = jnp.concatenate([w1_v[:, j * 128:(j + 1) * 128], ext], axis=0)
        w1T_v[j * 128:(j + 1) * 128, :] = blk.T
    b2r = jnp.broadcast_to(b2_v[...].astype(f32).reshape(1, D), (128, D))
    b2r = jnp.concatenate([b2r, jnp.zeros((128, 64), f32)], axis=1)
    b2c_v[...] = b2r.T[:D, :]

    zt = g_v[:, 512:640].T
    zrow = zt[64:65, :]
    hh = lax.broadcasted_iota(jnp.int32, (H, D), 0)
    dd = lax.broadcasted_iota(jnp.int32, (H, D), 1)
    zsel_v[...] = jnp.where(_head_of(dd) == hh, jnp.broadcast_to(zrow, (H, D)), 0.0).astype(bf)

    kvbd_v[...] = jnp.zeros((D, KP), bf)
    for j in range(5):
        e0 = j * 128
        ew = min(128, D - e0)
        h0 = e0 // DH
        h1 = (e0 + ew - 1) // DH
        r0 = (h0 * DH) // 16 * 16
        r1 = min(D, -(-((h1 + 1) * DH) // 16) * 16)
        gb = g_v[r0:r1, 0:D].astype(bf)
        kv = _dot(gb, wqkv_v[:, 1152 + e0:1152 + e0 + ew])
        dd = lax.broadcasted_iota(jnp.int32, (r1 - r0, ew), 0) + r0
        ee = lax.broadcasted_iota(jnp.int32, (r1 - r0, ew), 1) + e0
        kv = jnp.where(_head_of(dd) == _head_of(ee), kv, 0.0)
        kvbd_v[r0:r1, e0:e0 + ew] = kv.astype(bf)
    for j in range(5):
        d0 = j * 128
        dw = min(128, D - d0)
        h0 = d0 // DH
        h1 = (d0 + dw - 1) // DH
        e0 = (h0 * DH) // 128 * 128
        e1 = min(D, -(-((h1 + 1) * DH) // 128) * 128)
        mT = _dot(woT_v[:, e0:e1], kvbd_v[d0:d0 + dw, e0:e1], NT)
        mT_v[:, d0:d0 + dw] = mT.astype(bf)

    c_w2.wait()
    ones2 = (lax.broadcasted_iota(jnp.int32, (64, T2), 0) == 0).astype(bf)

    def attn(i):
        sl = slice(i * T2, (i + 1) * T2)
        pq = pq_v[:, sl]
        den = _dot(zsel_v[...], pq) + 1e-6
        inv = 1.0 / den
        rows = []
        for g in range(D // 8):
            h0 = (8 * g) // DH
            h1 = (8 * g + 7) // DH
            a = jnp.broadcast_to(inv[h0:h0 + 1, :], (8, T2))
            if h1 != h0:
                b = jnp.broadcast_to(inv[h1:h1 + 1, :], (8, T2))
                sub = lax.broadcasted_iota(jnp.int32, (8, T2), 0)
                a = jnp.where(sub < (h1 * DH - 8 * g), a, b)
            rows.append(a)
        inve = jnp.concatenate(rows, axis=0)
        pqs = (pq.astype(f32) * inve).astype(bf)
        h = x_v[:, sl].astype(f32) + _dot(mT_v[...], pqs)
        hn = _ln_T(h).astype(bf)
        hne = jnp.concatenate([hn, ones2], axis=0)
        acc0 = h + jnp.concatenate([b2c_v[...]] * (T2 // 128), axis=1)
        return hne, acc0

    def ffn(i, hne, acc):
        sl = slice(i * T2, (i + 1) * T2)
        for c in range(F // FC):
            h1 = _dot(w1T_v[c * FC:(c + 1) * FC, :], hne)
            r = jnp.maximum(h1, 0.0)
            r = (r * r).astype(bf)
            acc = acc + _dot(w2T_v[:, c * FC:(c + 1) * FC], r)
        out_v[:, sl] = acc.astype(bf)
        pltpu.make_async_copy(out_v.at[:, sl], out_hbm.at[:, sl], sem_o.at[i]).start()

    st = attn(0)
    for i in range(nb2):
        cur = st
        if i + 1 < nb2:
            st = attn(i + 1)
        ffn(i, *cur)
    for i in range(nb2):
        sl = slice(i * T2, (i + 1) * T2)
        pltpu.make_async_copy(out_v.at[:, sl], out_hbm.at[:, sl], sem_o.at[i]).wait()


@jax.jit
def pallas_sequential_preLN__linear_attn_block__dense_activation_squared_relu__prompt_kernel(A_x, A_wqkv, A_wo, B_x, B_w1, B_b1, B_w2, B_b2):
    xT = A_x.reshape(S, D).T
    w2T = B_w2.T
    anyspec = pl.BlockSpec(memory_space=pl.ANY)
    outT = pl.pallas_call(
        kern,
        out_shape=jax.ShapeDtypeStruct((D, S), bf),
        in_specs=[anyspec] * 7,
        out_specs=anyspec,
        scratch_shapes=[
            pltpu.VMEM((D, S), bf), pltpu.VMEM((D, 3 * D), bf), pltpu.VMEM((D, D), bf),
            pltpu.VMEM((D, F), bf), pltpu.VMEM((F // 128, 128), bf), pltpu.VMEM((D, F), bf), pltpu.VMEM((D,), bf),
            pltpu.VMEM((2 * D, D), bf), pltpu.VMEM((D, D), bf), pltpu.VMEM((F, KP), bf),
            pltpu.VMEM((D, KP), f32), pltpu.VMEM((D, S), bf), pltpu.VMEM((D, KP), bf), pltpu.VMEM((D, D), bf),
            pltpu.VMEM((H, D), bf), pltpu.VMEM((D, 128), f32), pltpu.VMEM((D, S), bf),
            pltpu.SemaphoreType.DMA((S // T1,)), pltpu.SemaphoreType.DMA((8,)), pltpu.SemaphoreType.DMA((S // T2,)),
        ],
        compiler_params=pltpu.CompilerParams(vmem_limit_bytes=100 * 1024 * 1024),
        name="blk",
    )(xT, A_wqkv, A_wo, B_w1, B_b1.reshape(F // 128, 128), w2T, B_b2)
    return outT.T.reshape(1, S, D)
```

```python
import os
import jax
import jax.numpy as jnp
from jax import lax
import jax.experimental.pallas as pl
import jax.experimental.pallas.tpu as pltpu

S, D, F, H, DH = 2048, 576, 4608, 32, 18
KP = 640
bf = jnp.bfloat16
f32 = jnp.float32
NN = (((1,), (0,)), ((), ()))
NT = (((1,), (1,)), ((), ()))

T1 = 512
T2 = 256
FC = 512
HF = FC // 2
HT = T2 // 2
NC = F // FC
HD = D // 2
OUT_PTS = tuple(int(c) for c in os.environ.get("OUT_PTS", "0,1,2,3,4,5,6,7").split(","))
ATT_MODE = os.environ.get("ATT_MODE", "pre")


def _dot(a, b, dims=NN):
    return lax.dot_general(a, b, dims, preferred_element_type=f32)


def _ln_T(x):
    m = jnp.sum(x, axis=0, keepdims=True) * (1.0 / D)
    xc = x - m
    v = jnp.sum(xc * xc, axis=0, keepdims=True) * (1.0 / D)
    return xc * lax.rsqrt(v + 1e-5)


def _phi(t):
    return jnp.where(t > 0, t + 1.0, jnp.exp(t)) + 1e-6


def _head_of(idx):
    return lax.shift_right_logical(idx * 3641, 16)


def _sA(a11, a12, a21, a22):
    return [a11 + a22, a21 + a22, a11, a22, a11 + a12, a21 - a11, a12 - a22]


def _sB(b11, b12, b21, b22):
    return [b11 + b22, b11, b12 - b22, b21 - b11, b22, b11 + b12, b21 + b22]


def _sC(m):
    return (m[0] + m[3] - m[4] + m[6], m[2] + m[4], m[1] + m[3], m[0] - m[1] + m[2] + m[5])


def kern(x_hbm, wqkv_hbm, wo_hbm, w1_hbm, b1_hbm, w2T_hbm, b2_hbm, out_hbm,
         x_v, wqkv_v, wo_v, w1_v, b1_v, w2T_v, b2_v,
         wqkT_v, woT_v, a1_v, t1_v, a2_v, g_v, pq_v, kvbd_v, mT_v, zsel_v, b2c_v, out_v,
         sem_w, sem_o):
    nb1 = S // T1
    nb2 = S // T2

    c_x0 = pltpu.make_async_copy(x_hbm.at[:, pl.ds(0, T1)], x_v.at[:, pl.ds(0, T1)], sem_w.at[7])
    c_x1 = pltpu.make_async_copy(x_hbm.at[:, pl.ds(T1, S - T1)], x_v.at[:, pl.ds(T1, S - T1)], sem_w.at[8])
    c_wqk = pltpu.make_async_copy(wqkv_hbm.at[:, pl.ds(0, 1152)], wqkv_v.at[:, pl.ds(0, 1152)], sem_w.at[0])
    c_wv = pltpu.make_async_copy(wqkv_hbm.at[:, pl.ds(1152, 576)], wqkv_v.at[:, pl.ds(1152, 576)], sem_w.at[1])
    c_wo = pltpu.make_async_copy(wo_hbm, wo_v, sem_w.at[2])
    c_w1 = pltpu.make_async_copy(w1_hbm, w1_v, sem_w.at[3])
    c_w2 = pltpu.make_async_copy(w2T_hbm, w2T_v, sem_w.at[4])
    c_b1 = pltpu.make_async_copy(b1_hbm, b1_v, sem_w.at[5])
    c_b2 = pltpu.make_async_copy(b2_hbm, b2_v, sem_w.at[6])

    def prep_w1(c):
        rows = []
        for jj in range(FC // 128):
            j = c * (FC // 128) + jj
            ext = (lax.broadcasted_iota(jnp.int32, (64, 128), 0) == 0)
            ext = jnp.where(ext, jnp.broadcast_to(b1_v[j:j + 1, :].astype(f32), (64, 128)), 0.0).astype(bf)
            blk = jnp.concatenate([w1_v[:, j * 128:(j + 1) * 128], ext], axis=0)
            rows.append(blk.T)
        wt = jnp.concatenate(rows, axis=0)
        t1_v[c * FC:(c + 1) * FC, :] = wt[:, 512:640]
        wf = wt[:, :512].astype(f32)
        ops = _sA(wf[:HF, :256], wf[:HF, 256:], wf[HF:, :256], wf[HF:, 256:])
        for p in range(7):
            a1_v[(c * 7 + p) * HF:(c * 7 + p + 1) * HF, :] = ops[p].astype(bf)

    def prep_w2(c):
        wf = w2T_v[:, c * FC:(c + 1) * FC].astype(f32)
        ops = _sA(wf[:HD, :HF], wf[:HD, HF:], wf[HD:, :HF], wf[HD:, HF:])
        k = 0
        for p in range(7):
            if p in (2, 3):
                continue
            a2_v[k * HD:(k + 1) * HD, c * HF:(c + 1) * HF] = ops[p].astype(bf)
            k += 1

    def a2_op(c, p):
        if p == 2:
            return w2T_v[0:HD, c * FC:c * FC + HF]
        if p == 3:
            return w2T_v[HD:D, c * FC + HF:(c + 1) * FC]
        k = p if p < 2 else p - 2
        return a2_v[k * HD:(k + 1) * HD, c * HF:(c + 1) * HF]

    c_wqk.start()
    c_x0.start()
    c_wqk.wait()
    c_x0.wait()
    c_x1.start()
    c_w1.start(); c_wv.start(); c_wo.start(); c_b1.start(); c_b2.start()
    for j in range(9):
        wqkT_v[j * 128:(j + 1) * 128, :] = wqkv_v[:, j * 128:(j + 1) * 128].T

    ones_blk = (lax.broadcasted_iota(jnp.int32, (64, T1), 0) == 0).astype(bf)

    def ln1(i):
        x = x_v[:, i * T1:(i + 1) * T1].astype(f32)
        return _ln_T(x).astype(bf)

    def kpart(i, xn):
        return _phi(_dot(wqkT_v[D:, :], xn)).astype(bf)

    def qpart(i, xn):
        pq_v[:, i * T1:(i + 1) * T1] = _phi(_dot(wqkT_v[:D, :], xn)).astype(bf)

    def gpart(i, xn, pk):
        xe = jnp.concatenate([xn, ones_blk], axis=0)
        g = _dot(pk, xe, NT)
        if i == 0:
            g_v[...] = g
        else:
            g_v[...] += g

    xn0 = ln1(0)
    pk0 = kpart(0, xn0)
    qpart(0, xn0)
    c_x1.wait()
    xn1 = ln1(1)
    gpart(0, xn0, pk0)
    pk1 = kpart(1, xn1)
    qpart(1, xn1)
    xn2 = ln1(2)
    gpart(1, xn1, pk1)
    c_w1.wait(); c_wv.wait(); c_wo.wait(); c_b1.wait(); c_b2.wait()
    c_w2.start()
    pk2 = kpart(2, xn2)
    qpart(2, xn2)
    xn3 = ln1(3)
    for j in range(4):
        woT_v[j * 128:(j + 1) * 128, :] = wo_v[:, j * 128:(j + 1) * 128].T
    woT_v[512:576, :] = wo_v[:, 448:576].T[64:, :]
    b2r = jnp.broadcast_to(b2_v[...].astype(f32).reshape(1, D), (128, D))
    b2r = jnp.concatenate([b2r, jnp.zeros((128, 64), f32)], axis=1)
    b2c_v[...] = b2r.T[:D, :]
    for c in range(NC):
        prep_w1(c)
    gpart(2, xn2, pk2)
    pk3 = kpart(3, xn3)
    gpart(3, xn3, pk3)
    c_w2.wait()
    qpart(3, xn3)
    for c in range(NC):
        prep_w2(c)

    zt = g_v[:, 512:640].T
    zrow = zt[64:65, :]
    hh = lax.broadcasted_iota(jnp.int32, (H, D), 0)
    dd = lax.broadcasted_iota(jnp.int32, (H, D), 1)
    zsel_v[...] = jnp.where(_head_of(dd) == hh, jnp.broadcast_to(zrow, (H, D)), 0.0).astype(bf)

    kvbd_v[...] = jnp.zeros((D, KP), bf)
    for j in range(5):
        e0 = j * 128
        ew = min(128, D - e0)
        h0 = e0 // DH
        h1 = (e0 + ew - 1) // DH
        r0 = (h0 * DH) // 16 * 16
        r1 = min(D, -(-((h1 + 1) * DH) // 16) * 16)
        gb = g_v[r0:r1, 0:D].astype(bf)
        kv = _dot(gb, wqkv_v[:, 1152 + e0:1152 + e0 + ew])
        dd = lax.broadcasted_iota(jnp.int32, (r1 - r0, ew), 0) + r0
        ee = lax.broadcasted_iota(jnp.int32, (r1 - r0, ew), 1) + e0
        kv = jnp.where(_head_of(dd) == _head_of(ee), kv, 0.0)
        kvbd_v[r0:r1, e0:e0 + ew] = kv.astype(bf)
    for j in range(5):
        d0 = j * 128
        dw = min(128, D - d0)
        h0 = d0 // DH
        h1 = (d0 + dw - 1) // DH
        e0 = (h0 * DH) // 128 * 128
        e1 = min(D, -(-((h1 + 1) * DH) // 128) * 128)
        mT = _dot(woT_v[:, e0:e1], kvbd_v[d0:d0 + dw, e0:e1], NT)
        mT_v[:, d0:d0 + dw] = mT.astype(bf)

    ones2 = (lax.broadcasted_iota(jnp.int32, (64, T2), 0) == 0).astype(bf)

    def att_a(i):
        sl = slice(i * T2, (i + 1) * T2)
        pq = pq_v[:, sl]
        den = _dot(zsel_v[...], pq) + 1e-6
        inv = 1.0 / den
        rows = []
        for g in range(D // 8):
            h0 = (8 * g) // DH
            h1 = (8 * g + 7) // DH
            a = jnp.broadcast_to(inv[h0:h0 + 1, :], (8, T2))
            if h1 != h0:
                b = jnp.broadcast_to(inv[h1:h1 + 1, :], (8, T2))
                sub = lax.broadcasted_iota(jnp.int32, (8, T2), 0)
                a = jnp.where(sub < (h1 * DH - 8 * g), a, b)
            rows.append(a)
        inve = jnp.concatenate(rows, axis=0)
        return (pq.astype(f32) * inve).astype(bf)

    def att_b(i, pqs):
        sl = slice(i * T2, (i + 1) * T2)
        return x_v[:, sl].astype(f32) + _dot(mT_v[...], pqs)

    def att_c(i, h):
        hn = _ln_T(h)
        Bm = [b.astype(bf) for b in _sB(hn[:256, :HT], hn[:256, HT:], hn[256:512, :HT], hn[256:512, HT:])]
        tail = jnp.concatenate([hn[512:].astype(bf), ones2], axis=0)
        hres = h + jnp.concatenate([b2c_v[...]] * (T2 // 128), axis=1)
        return Bm, tail, hres

    def attn(i):
        return att_c(i, att_b(i, att_a(i)))

    def act(h):
        r = jnp.maximum(h, 0.0)
        return r * r

    def ffn(i, Bm, tail, hres, hooks):
        sl = slice(i * T2, (i + 1) * T2)
        M = [None] * 7

        def w1(c):
            m = [_dot(a1_v[(c * 7 + p) * HF:(c * 7 + p + 1) * HF, :], Bm[p]) for p in range(7)]
            tl = _dot(t1_v[c * FC:(c + 1) * FC, :], tail)
            return m, tl

        def vpu(m, tl):
            c11, c12, c21, c22 = _sC(m)
            r11 = act(c11 + tl[:HF, :HT]); r12 = act(c12 + tl[:HF, HT:])
            r21 = act(c21 + tl[HF:, :HT]); r22 = act(c22 + tl[HF:, HT:])
            return [b.astype(bf) for b in _sB(r11, r12, r21, r22)]

        def w2(c, R):
            for p in range(7):
                mm = _dot(a2_op(c, p), R[p])
                M[p] = mm if M[p] is None else M[p] + mm

        nxt = w1(0)
        for c in range(NC):
            cur = nxt
            if c + 1 < NC:
                nxt = w1(c + 1)
            if c in hooks:
                hooks[c]()
            w2(c, vpu(*cur))
        o11, o12, o21, o22 = _sC(M)
        o = jnp.concatenate([jnp.concatenate([o11, o12], axis=1), jnp.concatenate([o21, o22], axis=1)], axis=0)
        out_v[:, sl] = (o + hres).astype(bf)

    def ocopy(k):
        lo = 0 if k == 0 else (OUT_PTS[k - 1] + 1) * T2
        hi = (OUT_PTS[k] + 1) * T2
        return pltpu.make_async_copy(out_v.at[:, pl.ds(lo, hi - lo)], out_hbm.at[:, pl.ds(lo, hi - lo)], sem_o.at[k])

    st = attn(0)
    for i in range(nb2):
        cur = st
        hooks = {}
        box = {}
        if i + 1 < nb2:
            if ATT_MODE == "pre":
                st = attn(i + 1)
            else:
                hk = [int(c) for c in ATT_MODE.split(",")]
                def ha(i=i, box=box): box["a"] = att_a(i + 1)
                def hb(i=i, box=box): box["b"] = att_b(i + 1, box["a"])
                def hc(i=i, box=box): box["c"] = att_c(i + 1, box["b"])
                hooks = {hk[0]: ha, hk[1]: hb, hk[2]: hc}
        ffn(i, *cur, hooks)
        if hooks:
            st = box["c"]
        if i in OUT_PTS:
            ocopy(OUT_PTS.index(i)).start()
    for k in range(len(OUT_PTS)):
        ocopy(k).wait()


@jax.jit
def pallas_sequential_preLN__linear_attn_block__dense_activation_squared_relu__prompt_kernel(A_x, A_wqkv, A_wo, B_x, B_w1, B_b1, B_w2, B_b2):
    xT = A_x.reshape(S, D).T
    w2T = B_w2.T
    anyspec = pl.BlockSpec(memory_space=pl.ANY)
    outT = pl.pallas_call(
        kern,
        out_shape=jax.ShapeDtypeStruct((D, S), bf),
        in_specs=[anyspec] * 7,
        out_specs=anyspec,
        scratch_shapes=[
            pltpu.VMEM((D, S), bf), pltpu.VMEM((D, 3 * D), bf), pltpu.VMEM((D, D), bf),
            pltpu.VMEM((D, F), bf), pltpu.VMEM((F // 128, 128), bf), pltpu.VMEM((D, F), bf), pltpu.VMEM((D,), bf),
            pltpu.VMEM((2 * D, D), bf), pltpu.VMEM((D, D), bf),
            pltpu.VMEM((NC * 7 * HF, 256), bf), pltpu.VMEM((F, 128), bf), pltpu.VMEM((5 * HD, F // 2), bf),
            pltpu.VMEM((D, KP), f32), pltpu.VMEM((D, S), bf), pltpu.VMEM((D, KP), bf), pltpu.VMEM((D, D), bf),
            pltpu.VMEM((H, D), bf), pltpu.VMEM((D, 128), f32), pltpu.VMEM((D, S), bf),
            pltpu.SemaphoreType.DMA((10,)), pltpu.SemaphoreType.DMA((S // T2,)),
        ],
        compiler_params=pltpu.CompilerParams(vmem_limit_bytes=100 * 1024 * 1024),
        name="blk",
    )(xT, A_wqkv, A_wo, B_w1, B_b1.reshape(F // 128, 128), w2T, B_b2)
    return outT.T.reshape(1, S, D)
```

```python
import os, json, contextlib
import jax
import jax.numpy as jnp
from jax import lax
import jax.experimental.pallas as pl
import jax.experimental.pallas.tpu as pltpu

S, D, F, H, DH = 2048, 576, 4608, 32, 18
KP = 640
bf = jnp.bfloat16
f32 = jnp.float32
u32 = jnp.uint32
NN = (((1,), (0,)), ((), ()))
NT = (((1,), (1,)), ((), ()))

T1 = int(os.environ.get("T1", "256"))
T2 = 256
FC = 512
HF = FC // 2
HT = T2 // 2
NC = F // FC
HD = D // 2
ONLY = os.environ.get("ONLY", "")
LNM = os.environ.get("LNM", "micro")
RG = int(os.environ.get("RG", "64"))
UB = int(os.environ.get("UB", "1"))
XA = int(os.environ.get('XA','1024'))
BC2 = int(os.environ.get('BC2','3'))
BD = int(os.environ.get('BD','5'))
BE = int(os.environ.get('BE','7'))
UA = int(os.environ.get("UA","4"))
P2N = int(os.environ.get('P2N','9'))
AORD = os.environ.get('AORD','b0 c b1 a b2 p')
NSP = int(os.environ.get('NSP','3'))
LNFIRST = int(os.environ.get('LNFIRST','1'))
TA = int(os.environ.get('TA','256'))
PW2 = int(os.environ.get('PW2','1'))
QDEF = int(os.environ.get('QDEF','1'))
SCOPE = int(os.environ.get("SCOPE", "0"))


def W(name, *cs):
    with (jax.named_scope(name) if SCOPE else contextlib.nullcontext()):
        for c in cs:
            c.wait()


def _dot(a, b, dims=NN):
    return lax.dot_general(a, b, dims, preferred_element_type=f32)


def _st(ref, r0, c0, val):
    nr, nc = val.shape
    ref[r0 // 2:(r0 + nr) // 2, c0:c0 + nc] = pltpu.bitcast(val, u32)


def _ld(ref, r0, nr, c0, nc):
    return pltpu.bitcast(ref[r0 // 2:(r0 + nr) // 2, c0:c0 + nc], bf)


def _ln_T(x):
    m = jnp.sum(x, axis=0, keepdims=True) * (1.0 / D)
    xc = x - m
    v = jnp.sum(xc * xc, axis=0, keepdims=True) * (1.0 / D)
    return xc * lax.rsqrt(v + 1e-5)


def _phi(t):
    return jnp.where(t > 0, t + 1.0, jnp.exp(t)) + 1e-6


def _head_of(idx):
    return lax.shift_right_logical(idx * 3641, 16)


def _sA(a11, a12, a21, a22):
    return [a11 + a22, a21 + a22, a11, a22, a11 + a12, a21 - a11, a12 - a22]


def _sB(b11, b12, b21, b22):
    return [b11 + b22, b11, b12 - b22, b21 - b11, b22, b11 + b12, b21 + b22]


def _sC(m):
    return (m[0] + m[3] - m[4] + m[6], m[2] + m[4], m[1] + m[3], m[0] - m[1] + m[2] + m[5])


def kern(x_hbm, wqkv_hbm, wo_hbm, w1_hbm, b1_hbm, w2T_hbm, b2_hbm, out_hbm,
         x_v, wqkv_v, wo_v, w1_v, b1_v, w2T_v, b2_v,
         wqkT_v, woT_v, a1_v, t1_v, a2_v, g_v, pq_v, kvbd_v, mT_v, zsel_v, b2c_v, out_v,
         bm_v, tl_v, h_v,
         sem_w, sem_o):
    nb1 = S // T1
    nb2 = S // T2

    def cp(src, dst, k, lo=None, n=None):
        if lo is None:
            return pltpu.make_async_copy(src, dst, sem_w.at[k])
        return pltpu.make_async_copy(src.at[:, pl.ds(lo, n)], dst.at[:, pl.ds(lo, n)], sem_w.at[k])
    c_x0 = cp(x_hbm, x_v, 0, 0, 256)
    c_wk = cp(wqkv_hbm, wqkv_v, 1, 512, 640)
    c_wq = cp(wqkv_hbm, wqkv_v, 2, 0, 512)
    c_xa = cp(x_hbm, x_v, 3, 256, XA - 256)
    c_xb = cp(x_hbm, x_v, 4, XA, S - XA)
    c_wv = cp(wqkv_hbm, wqkv_v, 5, 1152, 576)
    c_wo = cp(wo_hbm, wo_v, 6)
    c_b1 = cp(b1_hbm, b1_v, 7)
    c_b2 = cp(b2_hbm, b2_v, 8)
    c_w1 = cp(w1_hbm, w1_v, 9)
    c_w2 = cp(w2T_hbm, w2T_v, 10)

    def prep_w1(c):
        def tile(jj, kk):
            j = c * (FC // 128) + jj
            return w1_v[kk * 128:(kk + 1) * 128, j * 128:(j + 1) * 128].T
        for jj in range(2):
            for kk in range(2):
                tl = [tile(jj, kk), tile(jj, kk + 2), tile(jj + 2, kk), tile(jj + 2, kk + 2)]
                for r0 in range(0, 128, 32):
                    q = [t[r0:r0 + 32] for t in tl]
                    ops = _sA(*[t.astype(f32) for t in q])
                    for p in range(7):
                        v = q[0] if p == 2 else q[3] if p == 3 else ops[p].astype(bf)
                        _st(a1_v, (c * 7 + p) * HF + jj * 128 + r0, kk * 128, v)
        for jj in range(4):
            j = c * (FC // 128) + jj
            ext = (lax.broadcasted_iota(jnp.int32, (64, 128), 0) == 0)
            ext = jnp.where(ext, jnp.broadcast_to(b1_v[j:j + 1, :].astype(f32), (64, 128)), 0.0).astype(bf)
            blk = jnp.concatenate([w1_v[512:D, j * 128:(j + 1) * 128], ext], axis=0)
            _st(t1_v, j * 128, 0, blk.T)

    def prep_w2(c):
        for r0 in range(0, HD, 32):
            q = [w2T_v[r0 + a:r0 + a + 32, c * FC + b:c * FC + b + HF].astype(f32) for a in (0, HD) for b in (0, HF)]
            ops = _sA(*q)
            k = 0
            for p in range(7):
                if p in (2, 3):
                    continue
                _st(a2_v, k * HD + r0, c * HF, ops[p].astype(bf))
                k += 1

    def a2_op(c, p):
        if p == 2:
            return w2T_v[0:HD, c * FC:c * FC + HF]
        if p == 3:
            return w2T_v[HD:D, c * FC + HF:(c + 1) * FC]
        k = p if p < 2 else p - 2
        return _ld(a2_v, k * HD, HD, c * HF, HF)

    def ln1(t0, n):
        return _ln_T(x_v[:, t0:t0 + n].astype(f32)).astype(bf)

    def kpart(xn):
        return _phi(_dot(_ld(wqkT_v, D, D, 0, D), xn)).astype(bf)

    def qpart(t0, xn):
        _st(pq_v, 0, t0, _phi(_dot(_ld(wqkT_v, 0, D, 0, D), xn)).astype(bf))

    def gpart(first, xn, pk):
        n = xn.shape[1]
        ones_blk = (lax.broadcasted_iota(jnp.int32, (64, n), 0) == 0).astype(bf)
        xe = jnp.concatenate([xn, ones_blk], axis=0)
        g = _dot(pk, xe, NT)
        if first:
            g_v[...] = g
        else:
            g_v[...] += g

    def phase1():
        for c in (c_x0, c_wk, c_wq, c_xa, c_xb, c_wv, c_wo, c_b1, c_b2, c_w1, c_w2):
            c.start()
        W("B_x0", c_x0)
        xn = {0: ln1(0, 256)}
        W("B_wk", c_wk)
        for j in range(4, 9):
            _st(wqkT_v, j * 128, 0, wqkv_v[:, j * 128:(j + 1) * 128].T)
        gpart(True, xn[0], kpart(xn[0]))
        W("B_wq", c_wq, c_xa)
        for j in range(4):
            _st(wqkT_v, j * 128, 0, wqkv_v[:, j * 128:(j + 1) * 128].T)
        nb = S // 256
        nA = XA // 256
        xn[1] = ln1(256, 256)
        qpart(0, xn[0])

        def block(i, mid=None, lnnext=True):
            pk = kpart(xn[i])
            qpart(i * 256, xn[i])
            if lnnext:
                xn[i + 1] = ln1((i + 1) * 256, 256)
            if mid:
                mid()
            gpart(False, xn[i], pk)
        for i in range(1, BC2):
            block(i)
        W("B_xb", c_xb, c_wv, c_wo, c_b1, c_b2)
        for j in range(4):
            _st(woT_v, j * 128, 0, wo_v[:, j * 128:(j + 1) * 128].T)
        _st(woT_v, 512, 0, wo_v[:, 448:576].T[64:, :])
        b2r = jnp.broadcast_to(b2_v[...].astype(f32).reshape(1, D), (128, D))
        b2r = jnp.concatenate([b2r, jnp.zeros((128, 64), f32)], axis=1)
        b2c_v[...] = b2r.T[:D, :]
        for i in range(BC2, BD):
            block(i)
        W("B_w1", c_w1)
        n1 = BE - BD
        for i in range(BD, BE):
            def mid(i=i):
                for c in range((i - BD) * NC // n1, (i - BD + 1) * NC // n1):
                    prep_w1(c)
            block(i, mid, lnnext=i + 1 < nb)
        W("B_w2", c_w2)
        for i in range(BE, nb):
            def mid(i=i):
                for c in range(P2N):
                    prep_w2(c)
            block(i, mid if i == nb - 1 else None, lnnext=i + 1 < nb)

    def transition():
        zt = g_v[:, 512:640].T
        zrow = zt[64:65, :]
        hh = lax.broadcasted_iota(jnp.int32, (H, D), 0)
        dd = lax.broadcasted_iota(jnp.int32, (H, D), 1)
        zsel_v[...] = jnp.where(_head_of(dd) == hh, jnp.broadcast_to(zrow, (H, D)), 0.0).astype(bf)
        kvbd_v[...] = jnp.zeros((D, KP), bf)
        for j in range(5):
            e0 = j * 128
            ew = min(128, D - e0)
            h0 = e0 // DH
            h1 = (e0 + ew - 1) // DH
            r0 = (h0 * DH) // 16 * 16
            r1 = min(D, -(-((h1 + 1) * DH) // 16) * 16)
            gb = g_v[r0:r1, 0:D].astype(bf)
            kv = _dot(gb, wqkv_v[:, 1152 + e0:1152 + e0 + ew])
            dd = lax.broadcasted_iota(jnp.int32, (r1 - r0, ew), 0) + r0
            ee = lax.broadcasted_iota(jnp.int32, (r1 - r0, ew), 1) + e0
            kv = jnp.where(_head_of(dd) == _head_of(ee), kv, 0.0)
            kvbd_v[r0:r1, e0:e0 + ew] = kv.astype(bf)
        for j in range(5):
            d0 = j * 128
            dw = min(128, D - d0)
            h0 = d0 // DH
            h1 = (d0 + dw - 1) // DH
            e0 = (h0 * DH) // 128 * 128
            e1 = min(D, -(-((h1 + 1) * DH) // 128) * 128)
            mT = _dot(_ld(woT_v, 0, D, e0, e1 - e0), kvbd_v[d0:d0 + dw, e0:e1], NT)
            _st(mT_v, 0, d0, mT.astype(bf))

    def tsl(i, off=0, n=T2):
        if isinstance(i, int):
            return pl.ds(i * T2 + off, n)
        return pl.ds(pl.multiple_of(i * T2 + off, n), n)

    def att_a(i):
        pq = pltpu.bitcast(pq_v[:, tsl(i)], bf)
        den = _dot(zsel_v[...], pq) + 1e-6
        inv = 1.0 / den
        rows = []
        for g in range(D // 8):
            h0 = (8 * g) // DH
            h1 = (8 * g + 7) // DH
            a = jnp.broadcast_to(inv[h0:h0 + 1, :], (8, T2))
            if h1 != h0:
                b = jnp.broadcast_to(inv[h1:h1 + 1, :], (8, T2))
                sub = lax.broadcasted_iota(jnp.int32, (8, T2), 0)
                a = jnp.where(sub < (h1 * DH - 8 * g), a, b)
            rows.append(a)
        inve = jnp.concatenate(rows, axis=0)
        return (pq.astype(f32) * inve).astype(bf)

    def att_b(i, pqs):
        h = x_v[:, tsl(i)].astype(f32) + _dot(_ld(mT_v, 0, D, 0, D), pqs)
        h_v[:, tsl(i)] = h
        return h

    def att_c(i, h):
        ones2 = (lax.broadcasted_iota(jnp.int32, (64, T2), 0) == 0).astype(bf)
        hn = _ln_T(h)
        Bm = _sB(hn[:256, :HT], hn[:256, HT:], hn[256:512, :HT], hn[256:512, HT:])
        base = i * (7 * 128) if isinstance(i, int) else pl.multiple_of(i * (7 * 128), 128)
        for p in range(7):
            bm_v[pl.ds(base + p * 128, 128), :] = pltpu.bitcast(Bm[p].astype(bf), u32)
        tl_v[:, tsl(i)] = pltpu.bitcast(jnp.concatenate([hn[512:].astype(bf), ones2], axis=0), u32)

    def attention():
        def body(j, _):
            pq = [att_a(j * UA + u) for u in range(UA)]
            hs = []
            for u in range(UA):
                hs.append(att_b(j * UA + u, pq[u]))
                if u >= 1:
                    att_c(j * UA + u - 1, hs[u - 1])
            att_c(j * UA + UA - 1, hs[UA - 1])
            return 0
        if UA == nb2:
            body(0, 0)
        else:
            lax.fori_loop(0, nb2 // UA, body, 0)

    def act(h):
        r = jnp.maximum(h, 0.0)
        return r * r

    def ffn(i):
        M = [None] * 7
        base = pl.multiple_of(i * (7 * 128), 128)

        def w1(c):
            m = [_dot(_ld(a1_v, (c * 7 + p) * HF, HF, 0, 256),
                      pltpu.bitcast(bm_v[pl.ds(base + p * 128, 128), :], bf)) for p in range(7)]
            t = _dot(_ld(t1_v, c * FC, FC, 0, 128), pltpu.bitcast(tl_v[:, tsl(i)], bf))
            return m, t

        def vpu(m, t):
            c11, c12, c21, c22 = _sC(m)
            r11 = act(c11 + t[:HF, :HT]); r12 = act(c12 + t[:HF, HT:])
            r21 = act(c21 + t[HF:, :HT]); r22 = act(c22 + t[HF:, HT:])
            return [b.astype(bf) for b in _sB(r11, r12, r21, r22)]

        def w2(c, R):
            for p in range(7):
                mm = _dot(a2_op(c, p), R[p])
                M[p] = mm if M[p] is None else M[p] + mm

        nxt = w1(0)
        for c in range(NC):
            cur = nxt
            if c + 1 < NC:
                nxt = w1(c + 1)
            w2(c, vpu(*cur))
        o11, o12, o21, o22 = _sC(M)
        o = jnp.concatenate([jnp.concatenate([o11, o12], axis=1), jnp.concatenate([o21, o22], axis=1)], axis=0)
        o = o + h_v[:, tsl(i)] + jnp.concatenate([b2c_v[...]] * (T2 // 128), axis=1)
        out_v[:, tsl(i)] = o.astype(bf)

    def ocopy(i):
        return pltpu.make_async_copy(out_v.at[:, tsl(i)], out_hbm.at[:, tsl(i)], sem_o.at[i])

    if ONLY in ("", "p1"):
        phase1()
        transition()
        attention()
    if ONLY in ("", "p2"):
        def body(j, _):
            for u in range(UB):
                ffn(j * UB + u)
                ocopy(j * UB + u).start()
            return 0
        lax.fori_loop(0, nb2 // UB, body, 0)
        W("B_end", *[ocopy(i) for i in range(nb2)])


@jax.jit
def pallas_sequential_preLN__linear_attn_block__dense_activation_squared_relu__prompt_kernel(A_x, A_wqkv, A_wo, B_x, B_w1, B_b1, B_w2, B_b2):
    xT = A_x.reshape(S, D).T
    w2T = B_w2.T
    anyspec = pl.BlockSpec(memory_space=pl.ANY)
    outT = pl.pallas_call(
        kern,
        out_shape=jax.ShapeDtypeStruct((D, S), bf),
        in_specs=[anyspec] * 7,
        out_specs=anyspec,
        scratch_shapes=[
            pltpu.VMEM((D, S), bf), pltpu.VMEM((D, 3 * D), bf), pltpu.VMEM((D, D), bf),
            pltpu.VMEM((D, F), bf), pltpu.VMEM((F // 128, 128), bf), pltpu.VMEM((D, F), bf), pltpu.VMEM((D,), bf),
            pltpu.VMEM((D, D), u32), pltpu.VMEM((HD, D), u32),
            pltpu.VMEM((NC * 7 * HF // 2, 256), u32), pltpu.VMEM((F // 2, 128), u32), pltpu.VMEM((5 * HD // 2, F // 2), u32),
            pltpu.VMEM((D, KP), f32), pltpu.VMEM((HD, S), u32), pltpu.VMEM((D, KP), bf), pltpu.VMEM((HD, D), u32),
            pltpu.VMEM((H, D), bf), pltpu.VMEM((D, 128), f32), pltpu.VMEM((D, S), bf),
            pltpu.VMEM((S // T2 * 7 * 128, HT), u32), pltpu.VMEM((64, S), u32), pltpu.VMEM((D, S), f32),
            pltpu.SemaphoreType.DMA((11,)), pltpu.SemaphoreType.DMA((S // T2,)),
        ],
        compiler_params=pltpu.CompilerParams(vmem_limit_bytes=100 * 1024 * 1024),
        name="blk",
    )(xT, A_wqkv, A_wo, B_w1, B_b1.reshape(F // 128, 128), w2T, B_b2)
    return outT.T.reshape(1, S, D)
```

```python
import jax
import jax.numpy as jnp
from jax import lax
import jax.experimental.pallas as pl
import jax.experimental.pallas.tpu as pltpu

S, D, F, H, DH = 2048, 576, 4608, 32, 18
KP = 640
T = 256
FC = 512
HF, HT, HD = FC // 2, T // 2, D // 2
NC, NB = F // FC, S // T
XA = 768
UA = 4
bf, f32, u32 = jnp.bfloat16, jnp.float32, jnp.uint32
NN = (((1,), (0,)), ((), ()))
NT = (((1,), (1,)), ((), ()))


def _dot(a, b, dims=NN):
    return lax.dot_general(a, b, dims, preferred_element_type=f32)


def _st(ref, r0, c0, val):
    nr, nc = val.shape
    ref[r0 // 2:(r0 + nr) // 2, c0:c0 + nc] = pltpu.bitcast(val, u32)


def _ld(ref, r0, nr, c0, nc):
    return pltpu.bitcast(ref[r0 // 2:(r0 + nr) // 2, c0:c0 + nc], bf)


def _phi(t):
    return jnp.where(t > 0, t + 1.0, jnp.exp(t)) + 1e-6


def _head_of(idx):
    return lax.shift_right_logical(idx * 3641, 16)


def _iota(shape, axis):
    return lax.broadcasted_iota(jnp.int32, shape, axis)


def _sA(a11, a12, a21, a22):
    return [a11 + a22, a21 + a22, a11, a22, a11 + a12, a21 - a11, a12 - a22]


def _sB(b11, b12, b21, b22):
    return [b11 + b22, b11, b12 - b22, b21 - b11, b22, b11 + b12, b21 + b22]


def _sC(m):
    return (m[0] + m[3] - m[4] + m[6], m[2] + m[4], m[1] + m[3], m[0] - m[1] + m[2] + m[5])


def _block_kernel(x_hbm, wqkv_hbm, wo_hbm, w1_hbm, b1_hbm, w2T_hbm, b2_hbm, out_hbm,
                  x_v, wqkv_v, wo_v, w1_v, b1_v, w2T_v, b2_v,
                  wqkT_v, woT_v, a1_v, t1_v, a2_v, g_v, pq_v, kvbd_v, mT_v, zsel_v, b2c_v, out_v,
                  bm_v, tl_v, h_v, m1_v, sem_w, sem_o):
    def cp(src, dst, k, lo=None, n=None):
        if lo is None:
            return pltpu.make_async_copy(src, dst, sem_w.at[k])
        return pltpu.make_async_copy(src.at[:, pl.ds(lo, n)], dst.at[:, pl.ds(lo, n)], sem_w.at[k])

    c_x0 = cp(x_hbm, x_v, 0, 0, T)
    c_wk = cp(wqkv_hbm, wqkv_v, 1, 512, 640)
    c_wq = cp(wqkv_hbm, wqkv_v, 2, 0, 512)
    c_xa = cp(x_hbm, x_v, 3, T, XA - T)
    c_xb = cp(x_hbm, x_v, 4, XA, S - XA)
    c_wv = cp(wqkv_hbm, wqkv_v, 5, 2 * D, D)
    c_wo = cp(wo_hbm, wo_v, 6)
    c_b1 = cp(b1_hbm, b1_v, 7)
    c_b2 = cp(b2_hbm, b2_v, 8)
    c_w1 = cp(w1_hbm, w1_v, 9)
    c_w2 = cp(w2T_hbm, w2T_v, 10)

    def prep_w1(c):
        def tile(jj, kk):
            j = c * (FC // 128) + jj
            return w1_v[kk * 128:(kk + 1) * 128, j * 128:(j + 1) * 128].T
        for jj in range(2):
            for kk in range(2):
                tl = [tile(jj, kk), tile(jj, kk + 2), tile(jj + 2, kk), tile(jj + 2, kk + 2)]
                for r0 in range(0, 128, 32):
                    q = [t[r0:r0 + 32] for t in tl]
                    ops = _sA(*[t.astype(f32) for t in q])
                    for p in range(7):
                        v = q[0] if p == 2 else q[3] if p == 3 else ops[p].astype(bf)
                        _st(a1_v, (c * 7 + p) * HF + jj * 128 + r0, kk * 128, v)
        for jj in range(4):
            j = c * (FC // 128) + jj
            ext = jnp.where(_iota((64, 128), 0) == 0,
                            jnp.broadcast_to(b1_v[j:j + 1, :].astype(f32), (64, 128)), 0.0).astype(bf)
            blk = jnp.concatenate([w1_v[512:D, j * 128:(j + 1) * 128], ext], axis=0)
            _st(t1_v, j * 128, 0, blk.T)

    def prep_w2(c):
        for r0 in range(0, HD, 32):
            q = [w2T_v[r0 + a:r0 + a + 32, c * FC + b:c * FC + b + HF].astype(f32)
                 for a in (0, HD) for b in (0, HF)]
            ops = _sA(*q)
            for k, p in enumerate((0, 1, 4, 5, 6)):
                _st(a2_v, k * HD + r0, c * HF, ops[p].astype(bf))

    def a2_op(c, p):
        if p == 2:
            return w2T_v[0:HD, c * FC:c * FC + HF]
        if p == 3:
            return w2T_v[HD:D, c * FC + HF:(c + 1) * FC]
        return _ld(a2_v, (p if p < 2 else p - 2) * HD, HD, c * HF, HF)

    def ln1(i):
        x = x_v[:, i * T:(i + 1) * T].astype(f32)
        m = jnp.sum(x, axis=0, keepdims=True) * (1.0 / D)
        m1_v[:, i * T:(i + 1) * T] = jnp.broadcast_to(m, (8, T))
        xc = x - m
        v = jnp.sum(xc * xc, axis=0, keepdims=True) * (1.0 / D)
        return (xc * lax.rsqrt(v + 1e-5)).astype(bf)

    def kpart(xn):
        return _phi(_dot(_ld(wqkT_v, D, D, 0, D), xn)).astype(bf)

    def qpart(i, xn):
        pq = _phi(_dot(_ld(wqkT_v, 0, D, 0, D), xn)).astype(bf)
        for u in range(2):
            r0 = (2 * i + u) * D
            pq_v[r0:r0 + D, :] = pq[:, u * 128:(u + 1) * 128]

    def gpart(i, xn, pk):
        ones = (_iota((64, T), 0) == 0).astype(bf)
        g = _dot(pk, jnp.concatenate([xn, ones], axis=0), NT)
        if i == 0:
            g_v[...] = g
        else:
            g_v[...] += g

    for c in (c_x0, c_wk, c_wq, c_xa, c_xb, c_wv, c_wo, c_b1, c_b2, c_w1, c_w2):
        c.start()
    c_x0.wait()
    xn = {0: ln1(0)}
    c_wk.wait()
    for j in range(4, 9):
        _st(wqkT_v, j * 128, 0, wqkv_v[:, j * 128:(j + 1) * 128].T)
    gpart(0, xn[0], kpart(xn[0]))
    c_wq.wait()
    c_xa.wait()
    for j in range(4):
        _st(wqkT_v, j * 128, 0, wqkv_v[:, j * 128:(j + 1) * 128].T)
    xn[1] = ln1(1)
    qpart(0, xn[0])

    def block(i, mid=()):
        pk = kpart(xn[i])
        qpart(i, xn[i])
        if i + 1 < NB:
            xn[i + 1] = ln1(i + 1)
        for fn, c in mid:
            fn(c)
        gpart(i, xn[i], pk)

    nA = XA // T - 1
    for i in range(1, nA):
        block(i)
    for c in (c_xb, c_wv, c_wo, c_b1, c_b2):
        c.wait()
    for j in range(4):
        _st(woT_v, j * 128, 0, wo_v[:, j * 128:(j + 1) * 128].T)
    _st(woT_v, 512, 0, wo_v[:, 448:576].T[64:, :])
    b2r = jnp.broadcast_to(b2_v[...].astype(f32).reshape(1, D), (128, D))
    b2r = jnp.concatenate([b2r, jnp.zeros((128, 64), f32)], axis=1)
    b2c_v[...] = b2r.T[:D, :]
    for i in range(nA, 5):
        block(i)
    c_w1.wait()
    block(5, [(prep_w1, c) for c in range(0, 4)])
    block(6, [(prep_w1, c) for c in range(4, NC)])
    c_w2.wait()
    block(7, [(prep_w2, c) for c in range(NC)])

    zrow = g_v[:, 512:640].T[64:65, :]
    zsel_v[...] = jnp.where(_head_of(_iota((H, D), 1)) == _iota((H, D), 0),
                            jnp.broadcast_to(zrow, (H, D)), 0.0).astype(bf)
    kvbd_v[...] = jnp.zeros((D, KP), bf)
    for j in range(5):
        e0 = j * 128
        ew = min(128, D - e0)
        r0 = ((e0 // DH) * DH) // 16 * 16
        r1 = min(D, -(-(((e0 + ew - 1) // DH + 1) * DH) // 16) * 16)
        kv = _dot(g_v[r0:r1, 0:D].astype(bf), wqkv_v[:, 2 * D + e0:2 * D + e0 + ew])
        dd = _iota((r1 - r0, ew), 0) + r0
        ee = _iota((r1 - r0, ew), 1) + e0
        kvbd_v[r0:r1, e0:e0 + ew] = jnp.where(_head_of(dd) == _head_of(ee), kv, 0.0).astype(bf)
    for j in range(5):
        d0 = j * 128
        dw = min(128, D - d0)
        e0 = ((d0 // DH) * DH) // 128 * 128
        e1 = min(D, -(-(((d0 + dw - 1) // DH + 1) * DH) // 128) * 128)
        mb = _dot(_ld(woT_v, 0, D, e0, e1 - e0), kvbd_v[d0:d0 + dw, e0:e1], NT).astype(bf)
        cm = jnp.sum(mb.astype(f32), axis=0, keepdims=True) * (1.0 / D)
        ext = jnp.where(_iota((16, dw), 0) == 0, jnp.broadcast_to(cm, (16, dw)), 0.0)
        _st(mT_v, 0, d0, ext.astype(bf))
        _st(mT_v, 16, d0, mb)

    def tsl(i):
        return pl.ds(i * T if isinstance(i, int) else pl.multiple_of(i * T, T), T)

    def att_a(i):
        pq = jnp.concatenate([pq_v[pl.ds(pl.multiple_of((2 * i + u) * D, 16), D), :] for u in range(2)], axis=1)
        inv = 1.0 / (_dot(zsel_v[...], pq) + 1e-6)
        rows = []
        for g in range(D // 8):
            h0, h1 = (8 * g) // DH, (8 * g + 7) // DH
            a = jnp.broadcast_to(inv[h0:h0 + 1, :], (8, T))
            if h1 != h0:
                b = jnp.broadcast_to(inv[h1:h1 + 1, :], (8, T))
                a = jnp.where(_iota((8, T), 0) < (h1 * DH - 8 * g), a, b)
            rows.append(a)
        return (pq.astype(f32) * jnp.concatenate(rows, axis=0)).astype(bf)

    def att_b(i, pqs):
        e = _dot(_ld(mT_v, 0, D + 16, 0, D), pqs)
        h = x_v[:, tsl(i)].astype(f32) + e[16:]
        h_v[:, tsl(i)] = h
        hc = h - (m1_v[0:1, tsl(i)] + e[0:1])
        v = jnp.sum(hc * hc, axis=0, keepdims=True) * (1.0 / D)
        return hc, lax.rsqrt(v + 1e-5)

    def att_c(i, st):
        ones = (_iota((64, T), 0) == 0).astype(bf)
        hn = st[0] * st[1]
        Bm = _sB(hn[:256, :HT], hn[:256, HT:], hn[256:512, :HT], hn[256:512, HT:])
        base = pl.multiple_of(i * (7 * 256), 256)
        tl = jnp.concatenate([hn[512:].astype(bf), ones], axis=0)
        for p in range(7):
            bm_v[pl.ds(base + p * 256, 256), :] = Bm[p].astype(bf)
        for u in range(2):
            tl_v[pl.ds(pl.multiple_of((2 * i + u) * 128, 128), 128), :] = tl[:, u * 128:(u + 1) * 128]

    def att_body(j, carry):
        pq = [att_a(j * UA + u) for u in range(UA)]
        hs = []
        for u in range(UA):
            hs.append(att_b(j * UA + u, pq[u]))
            if u >= 1:
                att_c(j * UA + u - 1, hs[u - 1])
        att_c(j * UA + UA - 1, hs[UA - 1])
        return carry

    lax.fori_loop(0, NB // UA, att_body, 0)

    def act(h):
        r = jnp.maximum(h, 0.0)
        return r * r

    def ocopy(i):
        return pltpu.make_async_copy(out_v.at[:, tsl(i)], out_hbm.at[:, tsl(i)], sem_o.at[i])

    def ffn_body(i, carry):
        M = [None] * 7
        base = pl.multiple_of(i * (7 * 256), 256)

        def w1(c):
            m = [_dot(_ld(a1_v, (c * 7 + p) * HF, HF, 0, 256), bm_v[pl.ds(base + p * 256, 256), :])
                 for p in range(7)]
            tl = jnp.concatenate(
                [tl_v[pl.ds(pl.multiple_of((2 * i + u) * 128, 128), 128), :] for u in range(2)], axis=1)
            return m, _dot(_ld(t1_v, c * FC, FC, 0, 128), tl)

        def vpu(m, t):
            c11, c12, c21, c22 = _sC(m)
            r11, r12 = act(c11 + t[:HF, :HT]), act(c12 + t[:HF, HT:])
            r21, r22 = act(c21 + t[HF:, :HT]), act(c22 + t[HF:, HT:])
            return [b.astype(bf) for b in _sB(r11, r12, r21, r22)]

        nxt = w1(0)
        for c in range(NC):
            cur = nxt
            if c + 1 < NC:
                nxt = w1(c + 1)
            R = vpu(*cur)
            for p in range(7):
                mm = _dot(a2_op(c, p), R[p])
                M[p] = mm if M[p] is None else M[p] + mm
        o11, o12, o21, o22 = _sC(M)
        o = jnp.concatenate([jnp.concatenate([o11, o12], axis=1), jnp.concatenate([o21, o22], axis=1)], axis=0)
        o = o + h_v[:, tsl(i)] + jnp.concatenate([b2c_v[...]] * (T // 128), axis=1)
        out_v[:, tsl(i)] = o.astype(bf)
        ocopy(i).start()
        return carry

    lax.fori_loop(0, NB, ffn_body, 0)
    for i in range(NB):
        ocopy(i).wait()


@jax.jit
def pallas_sequential_preLN__linear_attn_block__dense_activation_squared_relu__prompt_kernel(
    A_x, A_wqkv, A_wo, B_x, B_w1, B_b1, B_w2, B_b2,
):
    del B_x
    anyspec = pl.BlockSpec(memory_space=pl.ANY)
    V = pltpu.VMEM
    outT = pl.pallas_call(
        _block_kernel,
        out_shape=jax.ShapeDtypeStruct((D, S), bf),
        in_specs=[anyspec] * 7,
        out_specs=anyspec,
        scratch_shapes=[
            V((D, S), bf), V((D, 3 * D), bf), V((D, D), bf),
            V((D, F), bf), V((F // 128, 128), bf), V((D, F), bf), V((D,), bf),
            V((D, D), u32), V((HD, D), u32),
            V((NC * 7 * HF // 2, 256), u32), V((F // 2, 128), u32), V((5 * HD // 2, F // 2), u32),
            V((D, KP), f32), V((S // 128 * D, 128), bf), V((D, KP), bf), V((HD + 8, D), u32),
            V((H, D), bf), V((D, 128), f32), V((D, S), bf),
            V((NB * 7 * 256, HT), bf), V((S, 128), bf), V((D, S), f32), V((8, S), f32),
            pltpu.SemaphoreType.DMA((11,)), pltpu.SemaphoreType.DMA((NB,)),
        ],
        compiler_params=pltpu.CompilerParams(vmem_limit_bytes=100 * 1024 * 1024),
        name="blk",
    )(A_x.reshape(S, D).T, A_wqkv, A_wo, B_w1, B_b1.reshape(F // 128, 128), B_w2.T, B_b2)
    return outT.T.reshape(1, S, D)
```
